```python
import os as _os
_os.environ.setdefault('JAX_PLATFORMS', 'cpu')
import jax
import jax.numpy as jnp

def _softmax(x, axis=-1):
    return jax.nn.softmax(x, axis=axis)

def _gelu(x):
    return jax.nn.gelu(x, approximate=True)

def _silu(x):
    return jax.nn.silu(x)

def _sigmoid(x):
    return jax.nn.sigmoid(x)

def _layernorm(x, axis=-1, eps=1e-05):
    m = jnp.mean(x, axis=axis, keepdims=True)
    v = jnp.var(x, axis=axis, keepdims=True)
    return (x - m) / jnp.sqrt(v + eps)

def _scatter_add(tgt, idx, src, axis=0):
    return tgt.at[idx].add(src)

def _segment_sum(src, seg, n):
    return jax.ops.segment_sum(src, seg, n)

class _Rng:

    def __init__(self, key):
        self._k = key

    def _next(self):
        self._k, sub = jax.random.split(self._k)
        return sub

    def normal(self, shape):
        return jax.random.normal(self._next(), shape, dtype=jnp.bfloat16)

    def randint(self, lo, hi, shape):
        return jax.random.randint(self._next(), shape, lo, hi, dtype=jnp.int32)

    def uniform(self, shape, lo=0.0, hi=1.0):
        return jax.random.uniform(self._next(), shape, jnp.bfloat16, lo, hi)

    def permutation(self, n):
        return jax.random.permutation(self._next(), n)
kernel_name = 'standalone__autoregressive_conv_wavenet__speech'

def setup_inputs():
    _rng = _Rng(jax.random.key(int.from_bytes(__import__("os").urandom(4), "little")))
    _w = lambda a: (lambda t: t.astype(jnp.bfloat16) if jnp.issubdtype(t.dtype, jnp.floating) else t)(jnp.asarray(a))
    B, T, D, K = (2, 4000, 512, 31)
    return {'x': _w((lambda *s: _rng.normal(s) * 0.05)(B, T, D)), 'w': _w((lambda *s: _rng.normal(s) * 0.05)(K, D, 2 * D)), 'w_o': _w((lambda *s: _rng.normal(s) * 0.05)(D, D))}

def reference(x, w, w_o):
    B, T, D = x.shape
    K = w.shape[0]
    dil = 2
    pad = (K - 1) * dil
    xp = jnp.pad(x, ((0, 0), (pad, 0), (0, 0)))
    h = jnp.einsum('btc,cd->btd', xp[:, pad:pad + T, :], w[0])
    for i in range(1, K):
        off = pad - i * dil
        h = h + jnp.einsum('btc,cd->btd', xp[:, off:off + T, :], w[i])
    f = h[..., :D].copy()
    g = h[..., D:].copy()
    z = jnp.tanh(f) * _sigmoid(g)
    return z @ w_o
```

```python
import jax
import jax.numpy as jnp
import jax.experimental.pallas as pl
import jax.experimental.pallas.tpu as pltpu


@jax.jit
def pallas_standalone__autoregressive_conv_wavenet__speech_kernel(
    x: jax.Array,
    w: jax.Array,
    w_o: jax.Array,
):
    B, T, D = x.shape
    K = w.shape[0]
    TT = 800
    HALO = 64
    nt = T // TT

    def kernel(xp_ref, xc_ref, w_ref, wo_ref, o_ref, xs_ref):
        t = pl.program_id(1)

        @pl.when(t == 0)
        def _():
            xs_ref[0:HALO, :] = jnp.zeros((HALO, D), jnp.bfloat16)

        @pl.when(t > 0)
        def _():
            xs_ref[0:HALO, :] = xp_ref[TT - HALO:TT, :]

        xs_ref[HALO:HALO + TT, :] = xc_ref[...]
        acc = None
        for i in range(K):
            off = HALO - 2 * i
            d = jnp.dot(xs_ref[off:off + TT, :], w_ref[i], preferred_element_type=jnp.float32)
            acc = d if acc is None else acc + d
        z = jnp.tanh(acc[:, :D]) * jax.nn.sigmoid(acc[:, D:])
        o_ref[...] = jnp.dot(z.astype(jnp.bfloat16), wo_ref[...],
                             preferred_element_type=jnp.float32).astype(o_ref.dtype)

    return pl.pallas_call(
        kernel,
        grid=(B, nt),
        in_specs=[
            pl.BlockSpec((None, TT, D), lambda b, t: (b, jnp.maximum(t - 1, 0), 0)),
            pl.BlockSpec((None, TT, D), lambda b, t: (b, t, 0)),
            pl.BlockSpec((K, D, 2 * D), lambda b, t: (0, 0, 0), pipeline_mode=pl.Buffered(1)),
            pl.BlockSpec((D, D), lambda b, t: (0, 0)),
        ],
        out_specs=pl.BlockSpec((None, TT, D), lambda b, t: (b, t, 0)),
        out_shape=jax.ShapeDtypeStruct((B, T, D), jnp.bfloat16),
        scratch_shapes=[pltpu.VMEM((HALO + TT, D), jnp.bfloat16)],
        compiler_params=pltpu.CompilerParams(
            dimension_semantics=("arbitrary", "arbitrary"),
            vmem_limit_bytes=100 * 1024 * 1024),
    )(x, x, w, w_o)
```

```python
import numpy as np
import ml_dtypes
import jax
import jax.numpy as jnp
from jax import lax
from jax.experimental import pallas as pl
from jax.experimental.pallas import tpu as pltpu

B, T, D, K = 2, 4000, 512, 31
N, H, F, NB = 96, 64, 48, 32
L = T // 2
U32 = jnp.uint32
BF = jnp.bfloat16
F32 = jnp.float32


def _pack_rows(a):
    b = a.astype(np.float32).astype(ml_dtypes.bfloat16).view(np.uint16).astype(np.uint32)
    return (b[0::2] | (b[1::2] << 16)).astype(np.uint32)


def _consts():
    th = 2 * np.pi * (np.arange(F) + 0.5) / N
    d = np.zeros((96, 128))
    m = np.arange(N)
    for fg in range(6):
        for i in range(8):
            f = 8 * fg + i
            d[16 * fg + i, :N] = np.cos(th[f] * m)
            d[16 * fg + 8 + i, :N] = -np.sin(th[f] * m)
    g = np.zeros((384, 128))
    k = np.arange(K)
    r = 0
    for cpl in range(2):
        for fg in range(6):
            for part in range(2):
                for h in range(2):
                    for i in range(8):
                        f = 8 * fg + i
                        v = np.cos(th[f] * k) if part == 0 else -np.sin(th[f] * k)
                        g[r, cpl * 64 + 2 * k + h] = v
                        r += 1
    c = np.zeros((64, 128))
    t = np.arange(H) + (N - H)
    for f in range(F):
        c[:, 2 * f] = (2.0 / N) * np.cos(th[f] * t)
        c[:, 2 * f + 1] = -(2.0 / N) * np.sin(th[f] * t)
    return _pack_rows(d), _pack_rows(g), _pack_rows(c)


PX = 68
PW = 68
PWK = 260
PY = 50
XS_ROWS = 1056
YH_ROWS = 128 * PY + 16


def make_fft(UW=64, UW0=16, UP=24, UI=64, UF=8, UX=25, UO=2, OB_ROWS=400, name="fft5"):
    dmat_np, gmat_np, cmat_np = _consts()

    def as_bf16(u):
        return pltpu.bitcast(u, BF)

    def pack(a, b):
        return pltpu.pack_elementwise([a, b], packed_dtype=BF)

    def kernel(d_ref, g_ref, c_ref, x_hbm, w_hbm, wo_hbm, o_hbm,
               XW, XS, XH, WB, WH, YH, ZB, WO, OB, sem_x, sem_w, sem_wo, sem_o):
        XWb = XW.bitcast(BF)
        WBb = WB.bitcast(BF)
        WOb = WO.bitcast(BF)

        def x_copy(ct, b):
            return pltpu.make_async_copy(
                x_hbm.at[b, :, pl.ds(ct * 128, 128)],
                XWb.at[pl.ds((ct * 2 + b) * T, T), :], sem_x.at[b])

        def w_copy(q, kt, k):
            col = q * 128 if isinstance(q, int) else pl.multiple_of(q * 128, 128)
            row = kt * 128 if isinstance(kt, int) else pl.multiple_of(kt * 128, 128)
            return pltpu.make_async_copy(
                w_hbm.at[k, pl.ds(row, 128), pl.ds(col, 128)],
                WBb.at[pl.ds(k * 2 * PWK + row, 128), :], sem_w.at[kt])

        def wf_copy(q, k, slot):
            col = q * 128 if isinstance(q, int) else pl.multiple_of(q * 128, 128)
            return pltpu.make_async_copy(
                w_hbm.at[k, :, pl.ds(col, 128)],
                WBb.at[pl.ds(pl.multiple_of((slot * 32 + k) * 2 * PWK, 8), D), :], sem_w.at[4 + slot])

        def w_start(q, kt):
            for k in range(K):
                w_copy(q, kt, k).start()

        def w_wait(q, kt):
            for k in range(K):
                w_copy(q, kt, k).wait()

        def wo_copy(nt):
            return pltpu.make_async_copy(
                wo_hbm.at[:, pl.ds(nt * 128, 128)],
                WOb.at[pl.ds(nt * D, D), :], sem_wo)

        def o_copy(slot, b, blk):
            return pltpu.make_async_copy(
                OB.at[slot], o_hbm.at[b, pl.ds(pl.multiple_of(blk * OB_ROWS, 16), OB_ROWS), :], sem_o.at[slot])

        w_start(0, 0)
        w_start(0, 1)

        zero8 = jnp.zeros((8, 128), U32)
        for slot in range(2):
            for i in range(32):
                WB[pl.ds((slot * 32 + K) * PWK + i * 8, 8), :] = zero8
        for tl in range(2):
            for i in range(16):
                YH[pl.ds(tl * YH_ROWS + 8 * i * PY + 48, 8, stride=PY), :] = zero8
                YH[pl.ds(tl * YH_ROWS + 8 * i * PY + 49, 8, stride=PY), :] = zero8
            YH[pl.ds(tl * YH_ROWS + 128 * PY, 8), :] = zero8
            YH[pl.ds(tl * YH_ROWS + 128 * PY + 8, 8), :] = zero8
        for p in range(2):
            for cb in range(8):
                base = (p * 8 + cb) * XS_ROWS
                for i in range(2):
                    XS[pl.ds(base + 8 * i, 8), :] = zero8
                for i in range(5):
                    XS[pl.ds(base + 1016 + 8 * i, 8), :] = zero8

        def w_groups(cpb, ng, slot):
            gmat = as_bf16(g_ref[...])
            kt = cpb >> 6
            row0 = cpb & 63
            wbase = kt * (F * PW) + row0
            for u0 in range(0, ng, 4):
                rs = []
                for u in range(u0, u0 + 4):
                    tile = jnp.concatenate(
                        [WB[pl.ds(slot * (32 * PWK) + cpb + (kg * 8 * PWK + 2 * u + cpl), 8, stride=PWK), :]
                         for cpl in range(2) for kg in range(4)], axis=0)
                    rs.append(jnp.dot(gmat, as_bf16(tile), preferred_element_type=F32))
                for cpl in range(2):
                    for fg in range(6):
                        o = (cpl * 6 + fg) * 32
                        for ui, r in enumerate(rs):
                            cp = 2 * (u0 + ui) + cpl
                            a0, a1 = r[o:o + 8], r[o + 8:o + 16]
                            b0, b1 = r[o + 16:o + 24], r[o + 24:o + 32]
                            for op, val in ((0, pack(a0, a1)), (1, pack(b0, b1)), (2, pack(a0 + b0, a1 + b1))):
                                off = ((op * 4 + cp // 64) * F + 8 * fg) * PW + cp % 64
                                WH[pl.ds(wbase + off, 8, stride=PW), :] = val

        def phase_xs(b):
            def body(ct, carry):
                cb = ct * 2 + b
                def inner(it, c2):
                    srcb = cb * L + it * (16 * UX)
                    dstb = cb * XS_ROWS + 16 + it * (8 * UX)
                    for u in range(UX):
                        e = XW[pl.ds(srcb + 16 * u, 8, stride=2), :]
                        o = XW[pl.ds(srcb + 16 * u + 1, 8, stride=2), :]
                        p0 = (e & jnp.uint32(0xFFFF)) | (o << 16)
                        p1 = (e >> 16) | (o & jnp.uint32(0xFFFF0000))
                        XS[pl.ds(dstb + 8 * u, 8), :] = p0
                        XS[pl.ds(dstb + (8 * XS_ROWS + 8 * u), 8), :] = p1
                    return c2
                lax.fori_loop(0, 125 // UX, inner, 0)
                return carry
            lax.fori_loop(0, 4, body, 0)

        def phase_f(b):
            def body(it, carry):
                dmat = as_bf16(d_ref[...])
                jp0 = it * UF
                xsb = b * XS_ROWS + 64 * jp0
                xhb = b * 32 + jp0
                for u in range(UF):
                    for p in range(2):
                        for ct in range(4):
                            off = (p * 8 + ct * 2) * XS_ROWS + 64 * u
                            t0 = XS[pl.ds(xsb + off, 64), :]
                            t1 = XS[pl.ds(xsb + off + 32, 64), :]
                            r0 = jnp.dot(dmat, as_bf16(t0), preferred_element_type=F32)
                            r1 = jnp.dot(dmat, as_bf16(t1), preferred_element_type=F32)
                            for fg in range(6):
                                xr0, xi0 = r0[16 * fg:16 * fg + 8], r0[16 * fg + 8:16 * fg + 16]
                                xr1, xi1 = r1[16 * fg:16 * fg + 8], r1[16 * fg + 8:16 * fg + 16]
                                for op, val in ((0, pack(xr0, xr1)), (1, pack(xi0, xi1)),
                                                (2, pack(xr0 + xi0, xr1 + xi1))):
                                    a = ((op * 4 + ct) * F + 8 * fg) * PX + p * 16 + u
                                    XH[pl.ds(xhb + a, 8, stride=PX), :] = val
                return carry
            lax.fori_loop(0, 16 // UF, body, 0)

        def phase_p(ybase):
            def body(it, carry):
                f0 = it * UP
                xb = f0 * PX
                wb = f0 * PW
                yb = ybase + f0
                for u in range(UP):
                    ks = []
                    for op in range(3):
                        acc = None
                        for kt in range(4):
                            xa = ((op * 4 + kt) * F + u) * PX
                            wa = ((op * 4 + kt) * F + u) * PW
                            d = jnp.dot(as_bf16(XH[pl.ds(xb + xa, 64), :]), as_bf16(WH[pl.ds(wb + wa, 64), :]),
                                        preferred_element_type=F32)
                            acc = d if acc is None else acc + d
                        ks.append(acc)
                    yr = ks[0] - ks[1]
                    yi = ks[2] - (ks[0] + ks[1])
                    y = pack(yr, yi)
                    for i in range(16):
                        YH[pl.ds(yb + (8 * i * PY + u), 8, stride=PY), :] = y[8 * i:8 * i + 8]
                return carry
            lax.fori_loop(0, F // UP, body, 0)

        def phase_i(ct):
            def body(it, carry):
                cmat = as_bf16(c_ref[...])
                idx0 = it * UI
                for u in range(UI):
                    hs = {}
                    for p in range(2):
                        for tl in range(2):
                            if UI == 64:
                                b, j = u >> 5, u & 31
                                yb = (b * 64 + j) * PY
                                zo = b * 2048 + 64 * j
                            else:
                                b, j0 = idx0 >> 5, idx0 & 31
                                yb = (b * 64 + j0) * PY + u * PY
                                zo = b * 2048 + 64 * j0 + 64 * u
                            rhs = as_bf16(YH[pl.ds(yb + (tl * YH_ROWS + p * 32 * PY), 64), :])
                            hs[p, tl] = jnp.dot(cmat, rhs, preferred_element_type=F32)
                    zs = [jnp.tanh(hs[p, 0]) * (0.5 * jnp.tanh(0.5 * hs[p, 1]) + 0.5) for p in range(2)]
                    z = pack(zs[0], zs[1])
                    ZB[pl.ds(ct * 4096 + zo, 64), :] = z
                return carry
            if UI == 64:
                body(0, 0)
            else:
                lax.fori_loop(0, 64 // UI, body, 0)

        def w0_body(it, carry):
            cpb = it * (2 * UW0)
            kt = cpb >> 6
            @pl.when((cpb & 63) == 0)
            def _():
                w_wait(0, kt)
                @pl.when(kt < 2)
                def _():
                    w_start(0, kt + 2)
                @pl.when(kt == 0)
                def _():
                    for ct in range(4):
                        x_copy(ct, 0).start()
                @pl.when(kt == 1)
                def _():
                    for ct in range(4):
                        x_copy(ct, 1).start()
                    for nt in range(4):
                        wo_copy(nt).start()
                @pl.when(kt == 2)
                def _():
                    for k in range(K):
                        wf_copy(4, k, 1).start()
            w_groups(cpb, UW0, 0)
            return carry
        with jax.named_scope("W0"):
            lax.fori_loop(0, 128 // UW0, w0_body, 0)
        for b in range(B):
            with jax.named_scope("wait_x"):
                for ct in range(4):
                    x_copy(ct, b).wait()
            with jax.named_scope("XS"):
                phase_xs(b)
            with jax.named_scope("F"):
                phase_f(b)

        def step(s, carry):
            q = (s >> 1) + 4 * (s & 1)
            sn = jnp.minimum(s + 1, 7)
            qn = (sn >> 1) + 4 * (sn & 1)

            @pl.when(s > 0)
            def _():
                with jax.named_scope("W"):
                    slot = s & 1
                    for k in range(K):
                        wf_copy(q, k, slot).wait()
                    nit = 128 // UW
                    for k in range(((K - 1) // nit) * nit, K):
                        wf_copy(qn, k, 1 - slot).start()
                    def wbody(it, c2):
                        for kk in range((K - 1) // nit):
                            wf_copy(qn, it + nit * kk, 1 - slot).start()
                        w_groups(it * (2 * UW), UW, slot)
                        return c2
                    if nit == 1:
                        wbody(0, 0)
                    else:
                        lax.fori_loop(0, nit, wbody, 0)
            with jax.named_scope("P"):
                phase_p((s & 1) * YH_ROWS)

            @pl.when((s & 1) == 1)
            def _():
                with jax.named_scope("I"):
                    phase_i(s >> 1)
            return carry
        lax.fori_loop(0, 8, step, 0)
        for k in range(K):
            wf_copy(7, k, 0).wait()

        for nt in range(4):
            wo_copy(nt).wait()
        NBLK = T // OB_ROWS
        def obody(it, carry):
            for u in range(UO):
                idx = it * UO + u
                b = (idx >= NBLK).astype(jnp.int32)
                blk = idx - b * NBLK
                slot = u if UO == 2 else idx & 1
                @pl.when(idx >= 2)
                def _():
                    o_copy(slot, b, blk).wait()
                zb = b * 2048 + blk * (OB_ROWS // 2)
                lhs = [as_bf16(ZB[pl.ds(zb + ct * 4096, OB_ROWS // 2), :]) for ct in range(4)]
                for nt in range(4):
                    acc = None
                    for kt in range(4):
                        d = jnp.dot(lhs[kt], as_bf16(WO[pl.ds(nt * 256 + kt * 64, 64), :]), preferred_element_type=F32)
                        acc = d if acc is None else acc + d
                    OB[slot, :, pl.ds(nt * 128, 128)] = acc.astype(BF)
                o_copy(slot, b, blk).start()
            return carry
        with jax.named_scope("O"):
            lax.fori_loop(0, B * NBLK // UO, obody, 0)
        for slot in range(2):
            o_copy(slot, 0, 0).wait()

    def fn(x, w, w_o):
        scratch = [
            pltpu.VMEM((8 * L, 128), U32),
            pltpu.VMEM((16 * XS_ROWS, 128), U32),
            pltpu.VMEM((12 * F * PX, 128), U32),
            pltpu.VMEM((64 * PWK, 128), U32),
            pltpu.VMEM((12 * F * PW, 128), U32),
            pltpu.VMEM((2 * YH_ROWS, 128), U32),
            pltpu.VMEM((8 * 2048, 128), U32),
            pltpu.VMEM((4 * 256, 128), U32),
            pltpu.VMEM((2, OB_ROWS, D), BF),
            pltpu.SemaphoreType.DMA((2,)), pltpu.SemaphoreType.DMA((6,)), pltpu.SemaphoreType.DMA,
            pltpu.SemaphoreType.DMA((2,)),
        ]
        return pl.pallas_call(
            kernel,
            out_shape=jax.ShapeDtypeStruct((B, T, D), BF),
            in_specs=[pl.BlockSpec(memory_space=pltpu.VMEM)] * 3 + [pl.BlockSpec(memory_space=pl.ANY)] * 3,
            out_specs=pl.BlockSpec(memory_space=pl.ANY),
            scratch_shapes=scratch,
            compiler_params=pltpu.CompilerParams(vmem_limit_bytes=120 * 1024 * 1024),
            name=name,
        )(jnp.asarray(dmat_np), jnp.asarray(gmat_np), jnp.asarray(cmat_np), x, w, w_o)
    fn.__name__ = name
    return fn


@jax.jit
def pallas_standalone__autoregressive_conv_wavenet__speech_kernel(
    x: jax.Array,
    w: jax.Array,
    w_o: jax.Array,
):
    return make_fft()(x, w, w_o)
```

```python
import math
import numpy as np
import ml_dtypes
import jax
import jax.numpy as jnp
from jax import lax
from jax.experimental import pallas as pl
from jax.experimental.pallas import tpu as pltpu

B, T, D, K = 2, 4000, 512, 31
N, H, F, NB = 96, 64, 48, 32
L = T // 2
U32 = jnp.uint32
BF = jnp.bfloat16
F32 = jnp.float32
EPS = 1e-12


def _lin(terms):
    terms = [(c, x) for c, x in terms if x is not None and abs(c) > EPS]
    if not terms:
        return None
    terms.sort(key=lambda t: (0 if t[0] > 0 else 1, 0 if abs(abs(t[0]) - 1.0) < EPS else 1))
    acc = None
    for c, x in terms:
        unit = abs(abs(c) - 1.0) < EPS
        if acc is None:
            acc = x if (unit and c > 0) else x * np.float32(c)
        else:
            v = x if unit else x * np.float32(abs(c))
            acc = acc + v if c > 0 else acc - v
    return acc


class C:
    __slots__ = ("r", "i")

    def __init__(self, r, i):
        self.r, self.i = r, i


class CN(C):
    __slots__ = ()


def _add(a, b):
    if a is None:
        return b
    if b is None:
        return a
    return a + b


def _sub(a, b):
    if b is None:
        return a
    if a is None:
        return -b
    return a - b


def cadd(a, b):
    return C(_add(a.r, b.r), _add(a.i, b.i))


def csub(a, b):
    return C(_sub(a.r, b.r), _sub(a.i, b.i))


def radix4(u0, u1, u2, u3):
    t0, t1 = cadd(u0, u2), csub(u0, u2)
    t2, t3 = cadd(u1, u3), csub(u1, u3)
    v0, v2 = cadd(t0, t2), csub(t0, t2)
    v1 = C(_add(t1.r, t3.i), _sub(t1.i, t3.r))
    v3 = C(_sub(t1.r, t3.i), _add(t1.i, t3.r))
    return v0, v1, v2, v3


def ctwiddle(v, num, den):
    num %= den
    if num == 0:
        return v
    if num * 4 == den:
        return CN(v.i, v.r)
    c, s = math.cos(2 * math.pi * num / den), math.sin(2 * math.pi * num / den)
    if abs(abs(c) - abs(s)) < EPS:
        h = abs(c)
        sc, ss = (1 if c > 0 else -1), (1 if s > 0 else -1)

        def comb(a, sa, b, sb):
            if sa > 0 and sb > 0:
                return a + b, 1
            if sa > 0 and sb < 0:
                return a - b, 1
            if sa < 0 and sb > 0:
                return b - a, 1
            return a + b, -1
        re, s1 = comb(v.r, sc, v.i, ss)
        im, s2 = comb(v.i, sc, v.r, -ss)
        return C(re * np.float32(h * s1), im * np.float32(h * s2))
    return C(_lin([(c, v.r), (s, v.i)]), _lin([(c, v.i), (-s, v.r)]))


def out_index(b, a):
    j = 12 * a + 4 * b + 1
    if j < 96:
        return (j - 1) // 2, False
    return (192 - j - 1) // 2, True


def bin_scale():
    c = np.ones(F, complex)
    for b in range(3):
        for a1 in range(4):
            f, cj = out_index(b, a1 + 12)
            assert cj
            c[f] = 1j
    return c


def pass2(z0, z1, z2, z3, b, a1):
    if isinstance(z2, CN):
        t0 = C(z0.r + z2.r, z0.i - z2.i)
        t1 = C(z0.r - z2.r, z0.i + z2.i)
    else:
        t0, t1 = cadd(z0, z2), csub(z0, z2)
    t2, t3 = cadd(z1, z3), csub(z1, z3)
    res = []
    for a2 in range(4):
        f, cj = out_index(b, a1 + 4 * a2)
        if a2 == 0:
            r, i = t0.r + t2.r, t0.i + t2.i
        elif a2 == 1:
            r, i = t1.r + t3.i, t1.i - t3.r
        elif a2 == 2:
            r, i = t0.r - t2.r, t2.i - t0.i
        else:
            r, i = t1.i + t3.r, t1.r - t3.i
        res.append((f, r, i))
    return res


def _pack_rows(a):
    b = a.astype(np.float32).astype(ml_dtypes.bfloat16).view(np.uint16).astype(np.uint32)
    return (b[0::2] | (b[1::2] << 16)).astype(np.uint32)


def _consts():
    th = 2 * np.pi * (np.arange(F) + 0.5) / N
    cs = bin_scale()
    d = np.zeros((96, 128))
    m = np.arange(N)
    for fg in range(6):
        for i in range(8):
            f = 8 * fg + i
            d[16 * fg + i, :N] = np.cos(th[f] * m)
            d[16 * fg + 8 + i, :N] = -np.sin(th[f] * m)
    g = np.zeros((384, 128))
    k = np.arange(K)
    r = 0
    for cpl in range(2):
        for fg in range(6):
            for part in range(2):
                for h in range(2):
                    for i in range(8):
                        f = 8 * fg + i
                        e = cs[f] * np.exp(-1j * th[f] * k)
                        g[r, cpl * 64 + 2 * k + h] = e.real if part == 0 else e.imag
                        r += 1
    c = np.zeros((64, 128))
    t = np.arange(H) + (N - H)
    for f in range(F):
        e = np.conj(cs[f]) * np.exp(1j * th[f] * t)
        c[:, 2 * f] = (2.0 / N) * e.real
        c[:, 2 * f + 1] = -(2.0 / N) * e.imag
    return _pack_rows(d), _pack_rows(g), _pack_rows(c)


PX = 68
PW = 68
PWK = 260
PY = 50
XS_ROWS = 1056
YH_ROWS = 128 * PY + 16


def sc_idx(h, b, a1, n2, part):
    return (((h * 3 + b) * 4 + a1) * 4 + n2) * 2 + part


def make_fft(NIT=4, MH=2, VLEAD=-0.01, UI=64, UF=8, UX=25, UO=2, OB_ROWS=400, NOBC=True, ORDER=('w00','w01','w02','x0','w03','w10','x1','w11','w20','w21'), name="fft9"):
    dmat_np, gmat_np, cmat_np = _consts()
    NP = 32 // NIT
    UP = F // NIT

    def as_bf16(u):
        return pltpu.bitcast(u, BF)

    def pack(a, b):
        return pltpu.pack_elementwise([a, b], packed_dtype=BF)

    def unpack(w, h):
        if h == 0:
            return lax.bitcast_convert_type(w << 16, F32)
        return lax.bitcast_convert_type(w & jnp.uint32(0xFFFF0000), F32)

    def p1_gen(WV, SC, row, scb, n2, h):
        taps = {}
        for n1 in range(4):
            for l in range(2):
                m = 4 * n1 + n2 + 16 * l
                if m < K:
                    taps[m] = unpack(WV[m, pl.ds(row, 8), :], h)
        for b in range(3):
            us = []
            for n1 in range(4):
                m0 = 4 * n1 + n2
                p1 = math.pi * m0 * (4 * b + 1) / 96
                p2 = math.pi * (m0 + 16) * (4 * b + 1) / 96
                x0, x1 = taps[m0], taps.get(m0 + 16)
                us.append(C(_lin([(math.cos(p1), x0), (math.cos(p2), x1)]),
                            _lin([(-math.sin(p1), x0), (-math.sin(p2), x1)])))
            vs = radix4(*us)
            for a1 in range(4):
                v = ctwiddle(vs[a1], n2 * a1, 16)
                SC[pl.ds(scb + 8 * sc_idx(h, b, a1, n2, 0), 8), :] = v.r
                SC[pl.ds(scb + 8 * sc_idx(h, b, a1, n2, 1), 8), :] = v.i
            yield

    def p2_gen(SC, WH, scb, whb, b, a1):
        res = []
        for h in range(2):
            zs = []
            for n2 in range(4):
                r = SC[pl.ds(scb + 8 * sc_idx(h, b, a1, n2, 0), 8), :]
                i = SC[pl.ds(scb + 8 * sc_idx(h, b, a1, n2, 1), 8), :]
                zs.append((CN if (n2 * a1) % 16 == 4 else C)(r, i))
            res.append(pass2(*zs, b, a1))
        for (f, r0, i0), (f1, r1, i1) in zip(*res):
            WH[pl.ds(whb + (0 * 4 * F + f) * PW, 8), :] = pack(r0 + i0, r1 + i1)
            WH[pl.ds(whb + (1 * 4 * F + f) * PW, 8), :] = pack(i0, i1)
            WH[pl.ds(whb + (2 * 4 * F + f) * PW, 8), :] = pack(r0, r1)
        yield

    def v_units(WV, SC, WHw, scb, whb, npos):
        gens = []
        for u in range(npos + 1):
            l1, l2 = [], []
            if u > 0:
                l1 = [p1_gen(WV, SC, (u - 1) * 8, scb + (u - 1) * 192 * 8, n2, h)
                      for n2 in range(4) for h in range(2)]
            if u < npos:
                l2 = [p2_gen(SC, WHw, scb + u * 192 * 8, whb + u * 8, b, a1) for b in range(3) for a1 in range(4)]
            flat1 = [g for g in l1 for _ in range(3)]
            for i in range(12):
                gens += flat1[2 * i:2 * i + 2] + l2[i:i + 1]
        return gens

    class Emitter:
        def __init__(self, gens, lead=0.0):
            self.gens, self.i, self.lead = gens, 0, lead

        def upto(self, frac):
            tgt = min(len(self.gens), int(math.ceil((frac + self.lead) * len(self.gens))))
            while self.i < tgt:
                next(self.gens[self.i])
                self.i += 1

    def kernel(d_ref, c_ref, x_hbm, w_hbm, wo_hbm, o_hbm,
               XW, XS, XH, WB, WH0, WH1, SC, YH, ZB, WO, OB, sem_x, sem_w, sem_wo, sem_o):
        XWb = XW.bitcast(BF)
        WBu = WB.bitcast(U32)
        WOb = WO.bitcast(BF)

        def qof(t):
            return (t >> 1) + 4 * (t & 1)

        def wview(slot, row, nrows):
            k0 = slot * K
            if not isinstance(row, int):
                row = pl.multiple_of(row, 8)
            return WBu.at[pl.ds(k0, K), pl.ds(row, nrows), :]

        def x_copy(ct, b):
            return pltpu.make_async_copy(
                x_hbm.at[b, :, pl.ds(ct * 128, 128)],
                XWb.at[pl.ds((ct * 2 + b) * T, T), :], sem_x.at[b])

        def wp_copy(t, slot, r0, nr, sem):
            q = qof(t)
            return pltpu.make_async_copy(
                w_hbm.at[:, pl.ds(r0, nr), pl.ds(q * 128, 128)],
                WB.at[pl.ds(slot * K, K), pl.ds(r0, nr), :], sem_w.at[sem])

        def wf_copy(t, slot):
            col = pl.multiple_of(qof(t) * 128, 128)
            return pltpu.make_async_copy(
                w_hbm.at[:, :, pl.ds(col, 128)], WB.at[pl.ds(slot * K, K)], sem_w.at[slot])

        pieces = {"w00": (0, 0, 0, 128, 3), "w01": (0, 0, 128, 128, 4), "w02": (0, 0, 256, 128, 5),
                  "w03": (0, 0, 384, 128, 6), "w10": (1, 1, 0, 128, 7), "w11": (1, 1, 128, 384, 8),
                  "w20": (2, 2, 0, 128, 9), "w21": (2, 2, 128, 384, 10)}

        def wo_copy(nt):
            return pltpu.make_async_copy(
                wo_hbm.at[:, pl.ds(nt * 128, 128)],
                WOb.at[pl.ds(nt * D, D), :], sem_wo)

        def o_copy(slot, b, blk):
            return pltpu.make_async_copy(
                OB.at[slot], o_hbm.at[b, pl.ds(pl.multiple_of(blk * OB_ROWS, 16), OB_ROWS), :], sem_o.at[slot])

        for name_ in ORDER:
            if name_[0] == "w" and name_ in pieces:
                wp_copy(*pieces[name_]).start()
            elif name_[0] == "x":
                for ct in range(4):
                    x_copy(ct, int(name_[1])).start()

        zero8 = jnp.zeros((8, 128), U32)
        for tl in range(2):
            for i in range(16):
                YH[pl.ds(tl * YH_ROWS + 8 * i * PY + 48, 8, stride=PY), :] = zero8
                YH[pl.ds(tl * YH_ROWS + 8 * i * PY + 49, 8, stride=PY), :] = zero8
            YH[pl.ds(tl * YH_ROWS + 128 * PY, 8), :] = zero8
            YH[pl.ds(tl * YH_ROWS + 128 * PY + 8, 8), :] = zero8
        for p in range(2):
            for cb in range(8):
                base = (p * 8 + cb) * XS_ROWS
                for i in range(2):
                    XS[pl.ds(base + 8 * i, 8), :] = zero8
                for i in range(5):
                    XS[pl.ds(base + 1016 + 8 * i, 8), :] = zero8

        def phase_xs(b):
            def body(ct, carry):
                cb = ct * 2 + b

                def inner(it, c2):
                    srcb = cb * L + it * (16 * UX)
                    dstb = cb * XS_ROWS + 16 + it * (8 * UX)
                    for u in range(UX):
                        e = XW[pl.ds(srcb + 16 * u, 8, stride=2), :]
                        o = XW[pl.ds(srcb + 16 * u + 1, 8, stride=2), :]
                        p0 = (e & jnp.uint32(0xFFFF)) | (o << 16)
                        p1 = (e >> 16) | (o & jnp.uint32(0xFFFF0000))
                        XS[pl.ds(dstb + 8 * u, 8), :] = p0
                        XS[pl.ds(dstb + (8 * XS_ROWS + 8 * u), 8), :] = p1
                    return c2
                lax.fori_loop(0, 125 // UX, inner, 0)
                return carry
            lax.fori_loop(0, 4, body, 0)

        def phase_fv(b, g2, slot1, g1):
            def body(it, carry):
                dmat = as_bf16(d_ref[...])
                jp0 = it * UF
                xsb = b * XS_ROWS + 64 * jp0
                xhb = b * 32 + jp0
                nit = 16 // UF
                npos = NP // nit
                cpg = g2 * (NP * 8) + it * (npos * 8)
                whb = (cpg >> 6) * (F * PW) + (cpg & 63)
                em = Emitter(v_units(wview(slot1, g1 * (NP * 8) + it * (npos * 8), npos * 8), SC, WH0,
                                     it * (npos * 192 * 8), whb, npos))
                nd, di = UF * 8, 0
                for u in range(UF):
                    for p in range(2):
                        for ct in range(4):
                            off = (p * 8 + ct * 2) * XS_ROWS + 64 * u
                            t0 = XS[pl.ds(xsb + off, 64), :]
                            t1 = XS[pl.ds(xsb + off + 32, 64), :]
                            r0 = jnp.dot(dmat, as_bf16(t0), preferred_element_type=F32)
                            r1 = jnp.dot(dmat, as_bf16(t1), preferred_element_type=F32)
                            for fg in range(6):
                                xr0, xi0 = r0[16 * fg:16 * fg + 8], r0[16 * fg + 8:16 * fg + 16]
                                xr1, xi1 = r1[16 * fg:16 * fg + 8], r1[16 * fg + 8:16 * fg + 16]
                                for op, val in ((0, pack(xr0, xr1)), (1, pack(xr0 + xi0, xr1 + xi1)),
                                                (2, pack(xi0 - xr0, xi1 - xr1))):
                                    a = ((op * 4 + ct) * F + 8 * fg) * PX + p * 16 + u
                                    XH[pl.ds(xhb + a, 8, stride=PX), :] = val
                            di += 1
                            em.upto(di / nd)
                em.upto(2.0)
                return carry
            lax.fori_loop(0, 16 // UF, body, 0)

        def phase_pv(s, WHr, WHw, ybase):
            slot1 = lax.rem(s + 1, 3)
            slot2 = lax.rem(s + 2, 3)

            def body(it, c):
                f0 = it * UP
                xb, wb, yb = f0 * PX, f0 * PW, ybase + f0
                last = it == NIT - 1
                g1 = jnp.where(last, 0, it + 1)
                cpg = it * (NP * 8)
                whb = (cpg >> 6) * (F * PW) + (cpg & 63)
                em = Emitter(v_units(wview(jnp.where(last, slot2, slot1), g1 * (NP * 8), NP * 8), SC, WHw, 0, whb, NP), VLEAD)
                nd = UP * 12 * MH
                di = 0
                MR = 64 // MH
                for u in range(UP):
                    for hh in range(MH):
                        ks = []
                        for op in range(3):
                            acc = None
                            for kt in range(4):
                                xa = ((op * 4 + kt) * F + u) * PX + hh * MR
                                wa = ((op * 4 + kt) * F + u) * PW
                                d = jnp.dot(as_bf16(XH[pl.ds(xb + xa, MR), :]),
                                            as_bf16(WHr[pl.ds(wb + wa, 64), :]), preferred_element_type=F32)
                                di += 1
                                acc = d if acc is None else acc + d
                                em.upto(di / nd)
                            ks.append(acc)
                            if op == 1:
                                yr = ks[0] - ks[1]
                        y = pack(yr, ks[0] + ks[2])
                        for i in range(16 // MH):
                            YH[pl.ds(yb + ((8 * i + hh * 2 * MR) * PY + u), 8, stride=PY), :] = y[8 * i:8 * i + 8]
                em.upto(2.0)
                return c
            lax.fori_loop(0, NIT, body, 0)

        def phase_i(ct):
            cmat = as_bf16(c_ref[...])
            for u in range(64):
                hs = {}
                b, j = u >> 5, u & 31
                for p in range(2):
                    for tl in range(2):
                        yb = (b * 64 + j) * PY
                        rhs = as_bf16(YH[pl.ds(yb + (tl * YH_ROWS + p * 32 * PY), 64), :])
                        hs[p, tl] = jnp.dot(cmat, rhs, preferred_element_type=F32)
                zs = [jnp.tanh(hs[p, 0]) * (0.5 * jnp.tanh(0.5 * hs[p, 1]) + 0.5) for p in range(2)]
                z = pack(zs[0], zs[1])
                ZB[pl.ds(ct * 4096 + b * 2048 + 64 * j, 64), :] = z

        wp_copy(*pieces["w00"]).wait()

        def pro1(u, carry):
            for n2 in range(4):
                for h in range(2):
                    for _ in p1_gen(wview(0, u * 8, 8), SC, 0, u * (192 * 8), n2, h):
                        pass
            return carry
        with jax.named_scope("V0"):
            lax.fori_loop(0, NP, pro1, 0)
        wp_copy(*pieces["w01"]).wait()
        wp_copy(*pieces["w02"]).wait()

        def vonly(g, carry):
            cpg = g * (NP * 8)
            whb = (cpg >> 6) * (F * PW) + (cpg & 63)
            Emitter(v_units(wview(0, (g + 1) * (NP * 8), NP * 8), SC, WH0, 0, whb, NP)).upto(2.0)
            return carry
        with jax.named_scope("Vonly"):
            lax.fori_loop(0, 2, vonly, 0)
        for b in range(B):
            with jax.named_scope("wait_x"):
                for ct in range(4):
                    x_copy(ct, b).wait()
            with jax.named_scope("XS"):
                phase_xs(b)
            with jax.named_scope("wait_w"):
                wp_copy(*pieces["w03" if b == 0 else "w10"]).wait()
            with jax.named_scope("FV"):
                if b == 0:
                    phase_fv(0, 2, 0, 3)
                else:
                    phase_fv(1, 3, 1, 0)
        wp_copy(*pieces["w11"]).wait()

        def dma_step(s, odd):
            if not odd:
                @pl.when(s == 0)
                def _():
                    wp_copy(*pieces["w20"]).wait()
                    for nt in range(4):
                        wo_copy(nt).start()

                @pl.when(jnp.logical_and(s > 0, s + 2 <= 7))
                def _():
                    wf_copy(s + 2, lax.rem(s + 2, 3)).wait()
            else:
                @pl.when(s == 1)
                def _():
                    wp_copy(*pieces["w21"]).wait()

                @pl.when(s + 2 <= 7)
                def _():
                    wf_copy(s + 2, lax.rem(s + 2, 3)).wait()

            @pl.when(s + 3 <= 7)
            def _():
                wf_copy(s + 3, lax.rem(s, 3)).start()

        def step2(c, carry):
            s = 2 * c
            dma_step(s, False)
            with jax.named_scope("PV"):
                phase_pv(s, WH0, WH1, 0)
            dma_step(s + 1, True)
            with jax.named_scope("PV"):
                phase_pv(s + 1, WH1, WH0, YH_ROWS)
            with jax.named_scope("I"):
                phase_i(c)
            return carry
        lax.fori_loop(0, 4, step2, 0)

        for nt in range(4):
            wo_copy(nt).wait()
        NBLK = T // OB_ROWS

        def obody(it, carry):
            for u in range(UO):
                idx = it * UO + u
                b = (idx >= NBLK).astype(jnp.int32)
                blk = idx - b * NBLK
                slot = u if UO == 2 else idx & 1

                @pl.when(idx >= 2)
                def _():
                    o_copy(slot, b, blk).wait()
                zb = b * 2048 + blk * (OB_ROWS // 2)
                lhs = [as_bf16(ZB[pl.ds(zb + ct * 4096, OB_ROWS // 2), :]) for ct in range(4)]
                for nt in range(4):
                    acc = None
                    for kt in range(4):
                        d = jnp.dot(lhs[kt], as_bf16(WO[pl.ds(nt * 256 + kt * 64, 64), :]), preferred_element_type=F32)
                        acc = d if acc is None else acc + d
                    OB[slot, :, pl.ds(nt * 128, 128)] = acc.astype(BF)
                o_copy(slot, b, blk).start()
            return carry
        with jax.named_scope("O"):
            lax.fori_loop(0, B * NBLK // UO, obody, 0)
        for slot in range(2):
            o_copy(slot, 0, 0).wait()

    def fn(x, w, w_o):
        scratch = [
            pltpu.VMEM((8 * L, 128), U32),
            pltpu.VMEM((16 * XS_ROWS, 128), U32),
            pltpu.VMEM((12 * F * PX, 128), U32),
            pltpu.VMEM((3 * K, D, 128), BF),
            pltpu.VMEM((12 * F * PW, 128), U32),
            pltpu.VMEM((12 * F * PW, 128), U32),
            pltpu.VMEM((NP * 192 * 8, 128), F32),
            pltpu.VMEM((2 * YH_ROWS, 128), U32),
            pltpu.VMEM((8 * 2048, 128), U32),
            pltpu.VMEM((4 * 256, 128), U32),
            pltpu.VMEM((2, OB_ROWS, D), BF),
            pltpu.SemaphoreType.DMA((2,)), pltpu.SemaphoreType.DMA((11,)), pltpu.SemaphoreType.DMA,
            pltpu.SemaphoreType.DMA((2,)),
        ]
        return pl.pallas_call(
            kernel,
            out_shape=jax.ShapeDtypeStruct((B, T, D), BF),
            in_specs=[pl.BlockSpec(memory_space=pltpu.VMEM)] * 2 + [pl.BlockSpec(memory_space=pl.ANY)] * 3,
            out_specs=pl.BlockSpec(memory_space=pl.ANY),
            scratch_shapes=scratch,
            compiler_params=pltpu.CompilerParams(vmem_limit_bytes=126 * 1024 * 1024, disable_bounds_checks=NOBC),
            name=name,
        )(jnp.asarray(dmat_np), jnp.asarray(cmat_np), x, w, w_o)
    fn.__name__ = name
    return fn


@jax.jit
def pallas_standalone__autoregressive_conv_wavenet__speech_kernel(
    x: jax.Array,
    w: jax.Array,
    w_o: jax.Array,
):
    return make_fft()(x, w, w_o)
```

```python
import math

import numpy as np
import jax
import jax.numpy as jnp
from jax import lax
from jax.experimental import pallas as pl
from jax.experimental.pallas import tpu as pltpu

B, T, D, K = 2, 4000, 512, 31
N, H, F, NB = 96, 64, 48, 32
L = T // 2
U32, BF, F32 = jnp.uint32, jnp.bfloat16, jnp.float32
EPS = 1e-12

PX = 72
PW = 72
PY = 50
XW_ROWS = L + 16
XSPLIT = 2048
XS_ROWS = 1056
YH_ROWS = 128 * PY + 16
NIT, MH, VLEAD = 2, 2, -0.005
NP, UP = 32 // NIT, F // NIT
UF = 8
UO, OB_ROWS = 5, 400


def _lin(terms):
    terms = [(c, x) for c, x in terms if x is not None and abs(c) > EPS]
    if not terms:
        return None
    terms.sort(key=lambda t: (0 if t[0] > 0 else 1, 0 if abs(abs(t[0]) - 1.0) < EPS else 1))
    acc = None
    for c, x in terms:
        unit = abs(abs(c) - 1.0) < EPS
        if acc is None:
            acc = x if (unit and c > 0) else x * np.float32(c)
        else:
            v = x if unit else x * np.float32(abs(c))
            acc = acc + v if c > 0 else acc - v
    return acc


class C:
    __slots__ = ("r", "i")

    def __init__(self, r, i):
        self.r, self.i = r, i


class CN(C):
    __slots__ = ()


def _add(a, b):
    if a is None:
        return b
    if b is None:
        return a
    return a + b


def _sub(a, b):
    if b is None:
        return a
    if a is None:
        return -b
    return a - b


def _cadd(a, b):
    return C(_add(a.r, b.r), _add(a.i, b.i))


def _csub(a, b):
    return C(_sub(a.r, b.r), _sub(a.i, b.i))


def _radix4(u0, u1, u2, u3):
    t0, t1 = _cadd(u0, u2), _csub(u0, u2)
    t2, t3 = _cadd(u1, u3), _csub(u1, u3)
    v0, v2 = _cadd(t0, t2), _csub(t0, t2)
    v1 = C(_add(t1.r, t3.i), _sub(t1.i, t3.r))
    v3 = C(_sub(t1.r, t3.i), _add(t1.i, t3.r))
    return v0, v1, v2, v3


def _ctwiddle(v, num, den):
    num %= den
    if num == 0:
        return v
    if num * 4 == den:
        return CN(v.i, v.r)
    c, s = math.cos(2 * math.pi * num / den), math.sin(2 * math.pi * num / den)
    if abs(abs(c) - abs(s)) < EPS:
        h = abs(c)
        sc, ss = (1 if c > 0 else -1), (1 if s > 0 else -1)

        def comb(a, sa, b, sb):
            if sa > 0 and sb > 0:
                return a + b, 1
            if sa > 0 and sb < 0:
                return a - b, 1
            if sa < 0 and sb > 0:
                return b - a, 1
            return a + b, -1
        re, s1 = comb(v.r, sc, v.i, ss)
        im, s2 = comb(v.i, sc, v.r, -ss)
        return C(re * np.float32(h * s1), im * np.float32(h * s2))
    return C(_lin([(c, v.r), (s, v.i)]), _lin([(c, v.i), (-s, v.r)]))


def _out_index(b, a):
    j = 12 * a + 4 * b + 1
    if j < 96:
        return (j - 1) // 2, False
    return (192 - j - 1) // 2, True


def _bin_scale():
    c = np.ones(F, complex)
    for b in range(3):
        for a1 in range(4):
            f, _ = _out_index(b, a1 + 12)
            c[f] = 1j
    return c


def _fft_pass2(z0, z1, z2, z3, b, a1):
    if isinstance(z2, CN):
        t0 = C(z0.r + z2.r, z0.i - z2.i)
        t1 = C(z0.r - z2.r, z0.i + z2.i)
    else:
        t0, t1 = _cadd(z0, z2), _csub(z0, z2)
    t2, t3 = _cadd(z1, z3), _csub(z1, z3)
    res = []
    for a2 in range(4):
        f, _ = _out_index(b, a1 + 4 * a2)
        if a2 == 0:
            r, i = t0.r + t2.r, t0.i + t2.i
        elif a2 == 1:
            r, i = t1.r + t3.i, t1.i - t3.r
        elif a2 == 2:
            r, i = t0.r - t2.r, t2.i - t0.i
        else:
            r, i = t1.i + t3.r, t1.r - t3.i
        res.append((f, r, i))
    return res


def _sc_idx(h, b, a1, n2, part):
    return (((h * 3 + b) * 4 + a1) * 4 + n2) * 2 + part


def _pack_rows(a):
    b = np.asarray(a.astype(np.float32), dtype=jnp.bfloat16).view(np.uint16).astype(np.uint32)
    return (b[0::2] | (b[1::2] << 16)).astype(np.uint32)


def _consts():
    th = 2 * np.pi * (np.arange(F) + 0.5) / N
    cs = _bin_scale()
    d = np.zeros((96, 128))
    m = np.arange(N)
    for fg in range(6):
        for i in range(8):
            f = 8 * fg + i
            d[16 * fg + i, :N] = np.cos(th[f] * m)
            d[16 * fg + 8 + i, :N] = -np.sin(th[f] * m)
    c = np.zeros((64, 128))
    t = np.arange(H) + (N - H)
    for f in range(F):
        e = np.conj(cs[f]) * np.exp(1j * th[f] * t)
        c[:, 2 * f] = (2.0 / N) * e.real
        c[:, 2 * f + 1] = -(2.0 / N) * e.imag
    return _pack_rows(d), _pack_rows(c)


_DMAT, _CMAT = _consts()


def _as_bf16(u):
    return pltpu.bitcast(u, BF)


def _pad64(t):
    return jnp.concatenate([t, jnp.zeros((16, 128), U32)], axis=0)


def _pack(a, b):
    return pltpu.pack_elementwise([a, b], packed_dtype=BF)


def _unpack(w, h):
    if h == 0:
        return lax.bitcast_convert_type(w << 16, F32)
    return lax.bitcast_convert_type(w & jnp.uint32(0xFFFF0000), F32)


def _mod3(x):
    return x - 3 * ((x * 11) >> 5)


class _Dep:
    v = None


def _p1_gen(WV, SC, row, scb, n2, h):
    taps = {}
    first = True
    for n1 in range(4):
        for l in range(2):
            m = 4 * n1 + n2 + 16 * l
            if m < K:
                wd = WV[m, pl.ds(row, 8), :]
                if _Dep.v is not None and first:
                    wd = wd | _Dep.v
                    first = False
                taps[m] = _unpack(wd, h)
    for b in (1, 2, 0):
        us = []
        for n1 in range(4):
            m0 = 4 * n1 + n2
            p1 = math.pi * m0 * (4 * b + 1) / 96
            p2 = math.pi * (m0 + 16) * (4 * b + 1) / 96
            x0, x1 = taps[m0], taps.get(m0 + 16)
            us.append(C(_lin([(math.cos(p1), x0), (math.cos(p2), x1)]),
                        _lin([(-math.sin(p1), x0), (-math.sin(p2), x1)])))
        vs = _radix4(*us)
        for a1 in range(4):
            v = _ctwiddle(vs[a1], n2 * a1, 16)
            SC[pl.ds(scb + 8 * _sc_idx(h, b, a1, n2, 0), 8), :] = v.r
            SC[pl.ds(scb + 8 * _sc_idx(h, b, a1, n2, 1), 8), :] = v.i
        yield


def _p2_gen(SC, WH, scb, whb, b, a1):
    res = []
    for h in range(2):
        zs = []
        for n2 in range(4):
            r = SC[pl.ds(scb + 8 * _sc_idx(h, b, a1, n2, 0), 8), :]
            i = SC[pl.ds(scb + 8 * _sc_idx(h, b, a1, n2, 1), 8), :]
            zs.append((CN if (n2 * a1) % 16 == 4 else C)(r, i))
        res.append(_fft_pass2(*zs, b, a1))
    for (f, r0, i0), (f1, r1, i1) in zip(*res):
        WH[pl.ds(whb + (0 * 4 * F + f) * PW, 8), :] = _pack(r0 + i0, r1 + i1)
        WH[pl.ds(whb + (1 * 4 * F + f) * PW, 8), :] = _pack(i0, i1)
        WH[pl.ds(whb + (2 * 4 * F + f) * PW, 8), :] = _pack(r0, r1)
    yield


def _v_units(WV, SC, WHw, scb, whb, npos, do1=True, do2=True):
    gens = []
    hn = [(n2, h) for h in range(2) for n2 in range(4)]
    for u in range(npos + 1):
        l1, l2 = [], []
        if u > 0 and do1:
            l1 = [_p1_gen(WV, SC, (u - 1) * 8, scb + (u - 1) * 192 * 8, n2, h) for n2, h in hn]
        if u < npos and do2:
            wo_ = (u >> 3) * (F * PW) + (u & 7) * 8
            l2 = [_p2_gen(SC, WHw, scb + u * 192 * 8, whb + wo_, b, a1) for b in range(3) for a1 in range(4)]
        flat1 = [g for g in l1 for _ in range(3)]
        n1s, n2s = len(flat1) // 12, len(l2) // 12
        for i in range(12):
            gens += l2[n2s * i:n2s * (i + 1)] + flat1[n1s * i:n1s * (i + 1)]
    return gens


class _Emitter:
    def __init__(self, gens, lead=0.0):
        self.gens, self.i, self.lead = gens, 0, lead

    def upto(self, frac):
        tgt = min(len(self.gens), int(math.ceil((frac + self.lead) * len(self.gens))))
        while self.i < tgt:
            next(self.gens[self.i])
            self.i += 1


def _kernel(d_ref, c_ref, x_hbm, w_hbm, wo_hbm, o_hbm,
            XW, XS, XH, WB, WH0, WH1, SC, YH, ZB, WO, OB, ZV, sem_x, sem_w, sem_wo, sem_o):
    XWb = XW.bitcast(BF)
    WBu = WB.bitcast(U32)
    WOb = WO.bitcast(BF)

    def qof(t):
        return (t >> 1) + 4 * (t & 1)

    def wview(slot, row, nrows):
        if not isinstance(row, int):
            row = pl.multiple_of(row, 8)
        return WBu.at[pl.ds(slot * K, K), pl.ds(row, nrows), :]

    def x_copy(ct, q):
        b, h = q >> 1, q & 1
        r0, nr, dst = (0, XSPLIT, 0) if h == 0 else (XSPLIT, T - XSPLIT, XSPLIT + 16)
        return pltpu.make_async_copy(
            x_hbm.at[b, pl.ds(r0, nr), pl.ds(ct * 128, 128)],
            XWb.at[pl.ds((ct * 2 + b) * 2 * XW_ROWS + dst, nr), :], sem_x.at[q])

    def w1_copy(q):
        return pltpu.make_async_copy(
            w_hbm.at[:, pl.ds(64 * q, 64), pl.ds(qof(1) * 128, 128)],
            WB.at[pl.ds(K, K), pl.ds(64 * q, 64), :], sem_w.at[10 + q])

    def xq_start(q):
        for ct in range(4):
            x_copy(ct, q).start()
        w1_copy(q).start()

    def w0_copy(r0, nr, sem):
        if not isinstance(r0, int):
            r0 = pl.multiple_of(r0, 128)
        return pltpu.make_async_copy(
            w_hbm.at[:, pl.ds(r0, nr), pl.ds(0, 128)],
            WB.at[pl.ds(0, K), pl.ds(r0, nr), :], sem_w.at[sem])

    def wh_copy(t, half, slot):
        q = qof(t)
        col = q * 128 if isinstance(q, int) else pl.multiple_of(q * 128, 128)
        return pltpu.make_async_copy(
            w_hbm.at[:, pl.ds(half * 256, 256), pl.ds(col, 128)],
            WB.at[pl.ds(slot * K, K), pl.ds(half * 256, 256), :], sem_w.at[slot * 2 + half])

    def wo_copy(nt):
        return pltpu.make_async_copy(
            wo_hbm.at[:, pl.ds(nt * 128, 128)], WOb.at[pl.ds(nt * D, D), :], sem_wo)

    def o_copy(slot, b, blk, par, nt=None):
        row = blk * OB_ROWS if isinstance(blk, int) else pl.multiple_of(blk * OB_ROWS, 16)
        if nt is None:
            return pltpu.make_async_copy(OB.at[slot], o_hbm.at[b, pl.ds(row, OB_ROWS), :], sem_o.at[par])
        return pltpu.make_async_copy(OB.at[slot, :, pl.ds(nt * 128, 128)],
                                     o_hbm.at[b, pl.ds(row, OB_ROWS), pl.ds(nt * 128, 128)], sem_o.at[par])

    w0_copy(0, 32, 6).start()
    w0_copy(32, 96, 14).start()
    for g in range(1, 4):
        w0_copy(128 * g, 128, 6 + g).start()
    xq_start(0)

    zero8 = jnp.zeros((8, 128), U32)
    ZV[...] = zero8
    for p in range(2):
        for cb in range(8):
            base = (p * 8 + cb) * XS_ROWS
            for i in range(2):
                XS[pl.ds(base + 8 * i, 8), :] = zero8
            for i in range(5):
                XS[pl.ds(base + 1016 + 8 * i, 8), :] = zero8

    def phase_xs(q):
        b, h = q >> 1, q & 1
        g0, ng, ux, off = (0, 64, 16, 0) if h == 0 else (64, 61, 61, 8)

        def body(ct, carry):
            cb = ct * 2 + b

            def inner(it, c2):
                srcb = cb * XW_ROWS + off + 16 * g0 + it * (16 * ux)
                dstb = cb * XS_ROWS + 16 + 8 * g0 + it * (8 * ux)
                for u in range(ux):
                    e = XW[pl.ds(srcb + 16 * u, 8, stride=2), :]
                    o = XW[pl.ds(srcb + 16 * u + 1, 8, stride=2), :]
                    XS[pl.ds(dstb + 8 * u, 8), :] = (e & jnp.uint32(0xFFFF)) | (o << 16)
                    XS[pl.ds(dstb + (8 * XS_ROWS + 8 * u), 8), :] = (e >> 16) | (o & jnp.uint32(0xFFFF0000))
                return c2
            lax.fori_loop(0, ng // ux, inner, 0)
            return carry
        lax.fori_loop(0, 4, body, 0)

    def phase_fv(q):
        b = q >> 1

        def body(it, carry):
            dmat = _as_bf16(d_ref[...])
            zero = ZV[...]
            jp0 = it * UF
            xsb = b * XS_ROWS + 64 * jp0
            xhb = b * 32 + jp0
            npos = 4
            pos0 = 8 * b + it * npos
            em = _Emitter(_v_units(wview(1, pos0 * 8, npos * 8), SC, WH0, pos0 * (192 * 8), 0, npos, do2=False))
            nd, di = UF * 8, 0
            for u in range(UF):
                for p in range(2):
                    for ct in range(4):
                        off = (p * 8 + ct * 2) * XS_ROWS + 64 * u
                        t0 = _pad64(XS[pl.ds(xsb + off, 48), :])
                        t1 = _pad64(XS[pl.ds(xsb + off + 32, 48), :])
                        r0 = jnp.dot(dmat, _as_bf16(t0), preferred_element_type=F32)
                        r1 = jnp.dot(dmat, _as_bf16(t1), preferred_element_type=F32)
                        for fg in range(6):
                            xr0, xi0 = r0[16 * fg:16 * fg + 8], r0[16 * fg + 8:16 * fg + 16]
                            xr1, xi1 = r1[16 * fg:16 * fg + 8], r1[16 * fg + 8:16 * fg + 16]
                            for op, val in ((0, _pack(xr0, xr1)), (1, _pack(xr0 + xi0, xr1 + xi1)),
                                            (2, _pack(xi0 - xr0, xi1 - xr1))):
                                a = ((op * 4 + ct) * F + 8 * fg) * PX + p * 16 + u
                                XH[pl.ds(xhb + a, 8, stride=PX), :] = val
                        di += 1
                        _Dep.v = lax.bitcast_convert_type(r0[0:8], U32) & zero
                        em.upto(di / nd)
            em.upto(2.0)
            _Dep.v = None
            return carry
        lax.fori_loop(q & 1, (q & 1) + 1, body, 0)

    def dma_half(s, half):
        if half == 0:
            @pl.when(s + 1 <= 7)
            def _():
                wh_copy(s + 1, 1, _mod3(s + 1)).wait()

            @pl.when(s + 3 <= 7)
            def _():
                wh_copy(s + 3, 0, _mod3(s)).start()
                wh_copy(s + 3, 1, _mod3(s)).start()
        else:
            @pl.when(s + 2 <= 7)
            def _():
                wh_copy(s + 2, 0, _mod3(s + 2)).wait()

    def phase_pv(s, WHr, WHw, ybase):
        slot1 = _mod3(s + 1)
        slot2 = _mod3(s + 2)

        def body(it, c):
            f0 = it * UP
            xb, wb, yb = f0 * PX, f0 * PW, ybase + f0
            last = it == NIT - 1
            g1 = jnp.where(last, 0, it + 1)
            cpg = it * (NP * 8)
            whb = (cpg >> 6) * (F * PW) + (cpg & 63)
            em = _Emitter(_v_units(wview(jnp.where(last, slot2, slot1), g1 * (NP * 8), NP * 8),
                                   SC, WHw, 0, whb, NP), VLEAD)
            nd = UP * 12 * MH
            di = 0
            MR = 64 // MH
            for u in range(UP):
                for hh in range(MH):
                    ks = {}
                    for op in (1, 2, 0):
                        ds = []
                        for kt in (0, 2, 1, 3):
                            xa = ((op * 4 + kt) * F + u) * PX + hh * MR
                            wa = ((op * 4 + kt) * F + u) * PW
                            ds.append(jnp.dot(_as_bf16(XH[pl.ds(xb + xa, MR), :]),
                                              _as_bf16(WHr[pl.ds(wb + wa, 64), :]), preferred_element_type=F32))
                            di += 1
                            em.upto(di / nd)
                        ks[op] = (ds[0] + ds[1]) + (ds[2] + ds[3])
                    y = _pack(ks[0] - ks[1], ks[0] + ks[2])
                    for i in range(16 // MH):
                        YH[pl.ds(yb + ((8 * i + hh * 2 * MR) * PY + u), 8, stride=PY), :] = y[8 * i:8 * i + 8]
            em.upto(2.0)
            return c

        def half_step(hs, c):
            @pl.when(hs == 0)
            def _():
                dma_half(s, 0)

            @pl.when(hs == 1)
            def _():
                dma_half(s, 1)
            lax.fori_loop(hs, hs + 1, body, 0)
            return c
        lax.fori_loop(0, NIT, half_step, 0)

    def phase_i(ct):
        cmat = _as_bf16(c_ref[...])
        for u in range(64):
            hs = {}
            b, j = u >> 5, u & 31
            for p in range(2):
                for tl in range(2):
                    yb = (b * 64 + j) * PY
                    rhs = _as_bf16(_pad64(YH[pl.ds(yb + (tl * YH_ROWS + p * 32 * PY), 48), :]))
                    hs[p, tl] = jnp.dot(cmat, rhs, preferred_element_type=F32)
            zs = [jnp.tanh(hs[p, 0]) * (0.5 * jnp.tanh(0.5 * hs[p, 1]) + 0.5) for p in range(2)]
            ZB[pl.ds(ct * 4096 + b * 2048 + 64 * j, 64), :] = _pack(zs[0], zs[1])

    def p1_loop(u0, u1):
        def body(u, carry):
            for g in _v_units(wview(0, u * 8, 8), SC, WH0, u * (192 * 8), 0, 1, do2=False):
                next(g)
            return carry
        lax.fori_loop(u0, u1, body, 0)

    w0_copy(0, 32, 6).wait()
    p1_loop(0, 2)
    w0_copy(32, 96, 14).wait()
    p1_loop(2, 8)
    xq_start(1)

    def vonly(g, carry):
        _Emitter(_v_units(wview(0, (g + 1) * 64, 64), SC, WH0, 0, g * (F * PW), 8)).upto(2.0)
        return carry

    def vstep(g, carry):
        w0_copy((g + 1) * 128, 128, 7 + g).wait()
        lax.fori_loop(g, g + 1, vonly, 0)

        @pl.when(g == 0)
        def _():
            xq_start(2)

        @pl.when(g == 1)
        def _():
            xq_start(3)
            wh_copy(1, 1, 1).start()
        return carry
    lax.fori_loop(0, 3, vstep, 0)
    _Emitter(_v_units(None, SC, WH0, 0, 3 * (F * PW), 8, do1=False)).upto(2.0)

    for q in range(4):
        for ct in range(4):
            x_copy(ct, q).wait()
        w1_copy(q).wait()
        phase_xs(q)
        if q == 1:
            wh_copy(2, 0, 2).start()
            wh_copy(2, 1, 2).start()
        phase_fv(q)
    for nt in range(4):
        wo_copy(nt).start()

    def step2(c, carry):
        s = 2 * c
        phase_pv(s, WH0, WH1, 0)
        phase_pv(s + 1, WH1, WH0, YH_ROWS)
        phase_i(c)
        return carry
    lax.fori_loop(0, 4, step2, 0)

    for nt in range(4):
        wo_copy(nt).wait()
    nblk = T // OB_ROWS

    def wait_out(par):
        for u in range(UO - 1):
            o_copy(par * UO + u, 0, 0, par).wait()
        for nt in range(4):
            o_copy(par * UO + UO - 1, 0, 0, par, nt).wait()

    def obody(it, carry):
        par = it & 1

        @pl.when(it >= 2)
        def _():
            wait_out(par)
        for u in range(UO):
            idx = it * UO + u
            b = (idx >= nblk).astype(jnp.int32)
            blk = idx - b * nblk
            slot = par * UO + u
            zb = b * 2048 + blk * (OB_ROWS // 2)
            lhs = [_as_bf16(ZB[pl.ds(zb + ct * 4096, OB_ROWS // 2), :]) for ct in range(4)]
            for nt in range(4):
                acc = None
                for kt in range(4):
                    d = jnp.dot(lhs[kt], _as_bf16(WO[pl.ds(nt * 256 + kt * 64, 64), :]),
                                preferred_element_type=F32)
                    acc = d if acc is None else acc + d
                OB[slot, :, pl.ds(nt * 128, 128)] = acc.astype(BF)
                if u == UO - 1:
                    o_copy(slot, b, blk, par, nt).start()
            if u < UO - 1:
                o_copy(slot, b, blk, par).start()
        return carry
    lax.fori_loop(0, B * nblk // UO, obody, 0)
    for par in range(2):
        wait_out(par)


def make_fft(name="wavenet_fft_conv"):
    def fn(x, w, w_o):
        scratch = [
            pltpu.VMEM((8 * XW_ROWS, 128), U32),
            pltpu.VMEM((16 * XS_ROWS, 128), U32),
            pltpu.VMEM((12 * F * PX + 64, 128), U32),
            pltpu.VMEM((3 * K, D, 128), BF),
            pltpu.VMEM((12 * F * PW, 128), U32),
            pltpu.VMEM((12 * F * PW, 128), U32),
            pltpu.VMEM((16 * 192 * 8, 128), F32),
            pltpu.VMEM((2 * YH_ROWS + 64, 128), U32),
            pltpu.VMEM((8 * 2048, 128), U32),
            pltpu.VMEM((4 * 256, 128), U32),
            pltpu.VMEM((2 * UO, OB_ROWS, D), BF),
            pltpu.VMEM((8, 128), U32),
            pltpu.SemaphoreType.DMA((4,)), pltpu.SemaphoreType.DMA((15,)), pltpu.SemaphoreType.DMA,
            pltpu.SemaphoreType.DMA((2,)),
        ]
        return pl.pallas_call(
            _kernel,
            out_shape=jax.ShapeDtypeStruct((B, T, D), BF),
            in_specs=[pl.BlockSpec(memory_space=pltpu.VMEM)] * 2 + [pl.BlockSpec(memory_space=pl.ANY)] * 3,
            out_specs=pl.BlockSpec(memory_space=pl.ANY),
            scratch_shapes=scratch,
            compiler_params=pltpu.CompilerParams(vmem_limit_bytes=126 * 1024 * 1024, disable_bounds_checks=True),
            name=name,
        )(jnp.asarray(_DMAT), jnp.asarray(_CMAT), x, w, w_o)
    fn.__name__ = name
    return fn


@jax.jit
def pallas_standalone__autoregressive_conv_wavenet__speech_kernel(
    x: jax.Array,
    w: jax.Array,
    w_o: jax.Array,
):
    assert x.shape == (B, T, D) and w.shape == (K, D, 2 * D) and w_o.shape == (D, D)
    return make_fft()(x, w, w_o)
```

```python
import math

import numpy as np
import jax
import jax.numpy as jnp
from jax import lax
from jax.experimental import pallas as pl
from jax.experimental.pallas import tpu as pltpu

B, T, D, K = 2, 4000, 512, 31
N, H, F, NB = 96, 64, 48, 32
L = T // 2
U32, BF, F32 = jnp.uint32, jnp.bfloat16, jnp.float32
EPS = 1e-12

PX = 72
PW = 72
PY = 50
XW_ROWS = L + 16
XSPLIT = 2048
XS_ROWS = 1056
YH_ROWS = 128 * PY + 16
NIT, MH, VLEAD = 2, 2, -0.005
NP, UP = 32 // NIT, F // NIT
UF = 8
UO, OB_ROWS = 5, 400


def _lin(terms):
    terms = [(c, x) for c, x in terms if x is not None and abs(c) > EPS]
    if not terms:
        return None
    terms.sort(key=lambda t: (0 if t[0] > 0 else 1, 0 if abs(abs(t[0]) - 1.0) < EPS else 1))
    acc = None
    for c, x in terms:
        unit = abs(abs(c) - 1.0) < EPS
        if acc is None:
            acc = x if (unit and c > 0) else x * np.float32(c)
        else:
            v = x if unit else x * np.float32(abs(c))
            acc = acc + v if c > 0 else acc - v
    return acc


class C:
    __slots__ = ("r", "i")

    def __init__(self, r, i):
        self.r, self.i = r, i


class CN(C):
    __slots__ = ()


def _add(a, b):
    if a is None:
        return b
    if b is None:
        return a
    return a + b


def _sub(a, b):
    if b is None:
        return a
    if a is None:
        return -b
    return a - b


def _cadd(a, b):
    return C(_add(a.r, b.r), _add(a.i, b.i))


def _csub(a, b):
    return C(_sub(a.r, b.r), _sub(a.i, b.i))


def _radix4(u0, u1, u2, u3):
    t0, t1 = _cadd(u0, u2), _csub(u0, u2)
    t2, t3 = _cadd(u1, u3), _csub(u1, u3)
    v0, v2 = _cadd(t0, t2), _csub(t0, t2)
    v1 = C(_add(t1.r, t3.i), _sub(t1.i, t3.r))
    v3 = C(_sub(t1.r, t3.i), _add(t1.i, t3.r))
    return v0, v1, v2, v3


def _ctwiddle(v, num, den):
    num %= den
    if num == 0:
        return v
    if num * 4 == den:
        return CN(v.i, v.r)
    c, s = math.cos(2 * math.pi * num / den), math.sin(2 * math.pi * num / den)
    if abs(abs(c) - abs(s)) < EPS:
        h = abs(c)
        sc, ss = (1 if c > 0 else -1), (1 if s > 0 else -1)

        def comb(a, sa, b, sb):
            if sa > 0 and sb > 0:
                return a + b, 1
            if sa > 0 and sb < 0:
                return a - b, 1
            if sa < 0 and sb > 0:
                return b - a, 1
            return a + b, -1
        re, s1 = comb(v.r, sc, v.i, ss)
        im, s2 = comb(v.i, sc, v.r, -ss)
        return C(re * np.float32(h * s1), im * np.float32(h * s2))
    return C(_lin([(c, v.r), (s, v.i)]), _lin([(c, v.i), (-s, v.r)]))


def _out_index(b, a):
    j = 12 * a + 4 * b + 1
    if j < 96:
        return (j - 1) // 2, False
    return (192 - j - 1) // 2, True


def _bin_scale():
    c = np.ones(F, complex)
    for b in range(3):
        for a1 in range(4):
            f, _ = _out_index(b, a1 + 12)
            c[f] = 1j
    return c


def _fft_pass2(z0, z1, z2, z3, b, a1):
    if isinstance(z2, CN):
        t0 = C(z0.r + z2.r, z0.i - z2.i)
        t1 = C(z0.r - z2.r, z0.i + z2.i)
    else:
        t0, t1 = _cadd(z0, z2), _csub(z0, z2)
    t2, t3 = _cadd(z1, z3), _csub(z1, z3)
    res = []
    for a2 in range(4):
        f, _ = _out_index(b, a1 + 4 * a2)
        if a2 == 0:
            r, i = t0.r + t2.r, t0.i + t2.i
        elif a2 == 1:
            r, i = t1.r + t3.i, t1.i - t3.r
        elif a2 == 2:
            r, i = t0.r - t2.r, t2.i - t0.i
        else:
            r, i = t1.i + t3.r, t1.r - t3.i
        res.append((f, r, i))
    return res


def _sc_idx(h, b, a1, n2, part):
    return (((h * 3 + b) * 4 + a1) * 4 + n2) * 2 + part


def _pack_rows(a):
    b = np.asarray(a.astype(np.float32), dtype=jnp.bfloat16).view(np.uint16).astype(np.uint32)
    return (b[0::2] | (b[1::2] << 16)).astype(np.uint32)


def _consts():
    th = 2 * np.pi * (np.arange(F) + 0.5) / N
    cs = _bin_scale()
    d = np.zeros((96, 128))
    m = np.arange(N)
    for fg in range(6):
        for i in range(8):
            f = 8 * fg + i
            d[16 * fg + i, :N] = np.cos(th[f] * m)
            d[16 * fg + 8 + i, :N] = -np.sin(th[f] * m)
    c = np.zeros((64, 128))
    t = np.arange(H) + (N - H)
    for f in range(F):
        e = np.conj(cs[f]) * np.exp(1j * th[f] * t)
        c[:, 2 * f] = (2.0 / N) * e.real
        c[:, 2 * f + 1] = -(2.0 / N) * e.imag
    return _pack_rows(d), _pack_rows(c)


_DMAT, _CMAT = _consts()


def _as_bf16(u):
    return pltpu.bitcast(u, BF)


def _pad64(t):
    return jnp.concatenate([t, jnp.zeros((16, 128), U32)], axis=0)


def _pack(a, b):
    return pltpu.pack_elementwise([a, b], packed_dtype=BF)


def _unpack(w, h):
    if h == 0:
        return lax.bitcast_convert_type(w << 16, F32)
    return lax.bitcast_convert_type(w & jnp.uint32(0xFFFF0000), F32)


def _mod3(x):
    return x - 3 * ((x * 11) >> 5)


class _Dep:
    v = None


def _p1_gen(WV, SC, row, scb, n2, h):
    taps = {}
    first = True
    for n1 in range(4):
        for l in range(2):
            m = 4 * n1 + n2 + 16 * l
            if m < K:
                wd = WV[m, pl.ds(row, 8), :]
                if _Dep.v is not None and first:
                    wd = wd | _Dep.v
                    first = False
                taps[m] = _unpack(wd, h)
    for b in (1, 2, 0):
        us = []
        for n1 in range(4):
            m0 = 4 * n1 + n2
            p1 = math.pi * m0 * (4 * b + 1) / 96
            p2 = math.pi * (m0 + 16) * (4 * b + 1) / 96
            x0, x1 = taps[m0], taps.get(m0 + 16)
            us.append(C(_lin([(math.cos(p1), x0), (math.cos(p2), x1)]),
                        _lin([(-math.sin(p1), x0), (-math.sin(p2), x1)])))
        vs = _radix4(*us)
        for a1 in range(4):
            v = _ctwiddle(vs[a1], n2 * a1, 16)
            SC[pl.ds(scb + 8 * _sc_idx(h, b, a1, n2, 0), 8), :] = v.r
            SC[pl.ds(scb + 8 * _sc_idx(h, b, a1, n2, 1), 8), :] = v.i
        yield


def _p2_gen(SC, WH, scb, whb, b, a1):
    res = []
    for h in range(2):
        zs = []
        for n2 in range(4):
            r = SC[pl.ds(scb + 8 * _sc_idx(h, b, a1, n2, 0), 8), :]
            i = SC[pl.ds(scb + 8 * _sc_idx(h, b, a1, n2, 1), 8), :]
            zs.append((CN if (n2 * a1) % 16 == 4 else C)(r, i))
        res.append(_fft_pass2(*zs, b, a1))
    for (f, r0, i0), (f1, r1, i1) in zip(*res):
        WH[pl.ds(whb + (0 * 4 * F + f) * PW, 8), :] = _pack(r0 + i0, r1 + i1)
        WH[pl.ds(whb + (1 * 4 * F + f) * PW, 8), :] = _pack(i0, i1)
        WH[pl.ds(whb + (2 * 4 * F + f) * PW, 8), :] = _pack(r0, r1)
    yield


def _v_units(WV, SC, WHw, scb, whb, npos, do1=True, do2=True):
    gens = []
    hn = [(n2, h) for h in range(2) for n2 in range(4)]
    for u in range(npos + 1):
        l1, l2 = [], []
        if u > 0 and do1:
            l1 = [_p1_gen(WV, SC, (u - 1) * 8, scb + (u - 1) * 192 * 8, n2, h) for n2, h in hn]
        if u < npos and do2:
            wo_ = (u >> 3) * (F * PW) + (u & 7) * 8
            l2 = [_p2_gen(SC, WHw, scb + u * 192 * 8, whb + wo_, b, a1) for b in range(3) for a1 in range(4)]
        flat1 = [g for g in l1 for _ in range(3)]
        n1s, n2s = len(flat1) // 12, len(l2) // 12
        for i in range(12):
            gens += l2[n2s * i:n2s * (i + 1)] + flat1[n1s * i:n1s * (i + 1)]
    return gens


class _Emitter:
    def __init__(self, gens, lead=0.0):
        self.gens, self.i, self.lead = gens, 0, lead

    def upto(self, frac):
        tgt = min(len(self.gens), int(math.ceil((frac + self.lead) * len(self.gens))))
        while self.i < tgt:
            next(self.gens[self.i])
            self.i += 1


def _kernel(d_ref, c_ref, x_hbm, w_hbm, wo_hbm, o_hbm,
            XW, XS, XH, WB, WH0, WH1, SC, YH, ZB, WO, OB, ZV, sem_x, sem_w, sem_wo, sem_o):
    XWb = XW.bitcast(BF)
    WBu = WB.bitcast(U32)
    WOb = WO.bitcast(BF)

    def qof(t):
        return (t >> 1) + 4 * (t & 1)

    def wview(slot, row, nrows):
        if not isinstance(row, int):
            row = pl.multiple_of(row, 8)
        return WBu.at[pl.ds(slot * K, K), pl.ds(row, nrows), :]

    def x_copy(ct, b, h):
        q = 2 * b + h
        r0, nr, dst = (0, XSPLIT, 0) if h == 0 else (XSPLIT, T - XSPLIT, XSPLIT + 16)
        return pltpu.make_async_copy(
            x_hbm.at[b, pl.ds(r0, nr), pl.ds(ct * 128, 128)],
            XWb.at[pl.ds((ct * 2 + b) * 2 * XW_ROWS + dst, nr), :], sem_x.at[q])

    def w1_copy(q):
        r0 = 64 * q if isinstance(q, int) else pl.multiple_of(64 * q, 64)
        return pltpu.make_async_copy(
            w_hbm.at[:, pl.ds(r0, 64), pl.ds(qof(1) * 128, 128)],
            WB.at[pl.ds(K, K), pl.ds(r0, 64), :], sem_w.at[10 + q])

    def xq_start(q):
        for ct in range(4):
            x_copy(ct, q >> 1, q & 1).start()
        w1_copy(q).start()

    def w0_copy(r0, nr, sem):
        if not isinstance(r0, int):
            r0 = pl.multiple_of(r0, 128)
        return pltpu.make_async_copy(
            w_hbm.at[:, pl.ds(r0, nr), pl.ds(0, 128)],
            WB.at[pl.ds(0, K), pl.ds(r0, nr), :], sem_w.at[sem])

    def wh_copy(t, half, slot):
        q = qof(t)
        col = q * 128 if isinstance(q, int) else pl.multiple_of(q * 128, 128)
        return pltpu.make_async_copy(
            w_hbm.at[:, pl.ds(half * 256, 256), pl.ds(col, 128)],
            WB.at[pl.ds(slot * K, K), pl.ds(half * 256, 256), :], sem_w.at[slot * 2 + half])

    def wo_copy(nt):
        return pltpu.make_async_copy(
            wo_hbm.at[:, pl.ds(nt * 128, 128)], WOb.at[pl.ds(nt * D, D), :], sem_wo)

    def o_copy(slot, b, blk, par, nt=None):
        row = blk * OB_ROWS if isinstance(blk, int) else pl.multiple_of(blk * OB_ROWS, 16)
        if nt is None:
            return pltpu.make_async_copy(OB.at[slot], o_hbm.at[b, pl.ds(row, OB_ROWS), :], sem_o.at[par])
        return pltpu.make_async_copy(OB.at[slot, :, pl.ds(nt * 128, 128)],
                                     o_hbm.at[b, pl.ds(row, OB_ROWS), pl.ds(nt * 128, 128)], sem_o.at[par])

    w0_copy(0, 32, 6).start()
    w0_copy(32, 96, 14).start()
    for g in range(1, 4):
        w0_copy(128 * g, 128, 6 + g).start()
    xq_start(0)

    zero8 = jnp.zeros((8, 128), U32)
    ZV[...] = zero8
    for p in range(2):
        for cb in range(8):
            base = (p * 8 + cb) * XS_ROWS
            for i in range(2):
                XS[pl.ds(base + 8 * i, 8), :] = zero8
            for i in range(5):
                XS[pl.ds(base + 1016 + 8 * i, 8), :] = zero8

    def phase_xs(b, h):
        g0, ng, ux, off = (0, 64, 16, 0) if h == 0 else (64, 61, 61, 8)

        def body(ct, carry):
            cb = ct * 2 + b

            def inner(it, c2):
                srcb = cb * XW_ROWS + off + 16 * g0 + it * (16 * ux)
                dstb = cb * XS_ROWS + 16 + 8 * g0 + it * (8 * ux)
                for u in range(ux):
                    e = XW[pl.ds(srcb + 16 * u, 8, stride=2), :]
                    o = XW[pl.ds(srcb + 16 * u + 1, 8, stride=2), :]
                    XS[pl.ds(dstb + 8 * u, 8), :] = (e & jnp.uint32(0xFFFF)) | (o << 16)
                    XS[pl.ds(dstb + (8 * XS_ROWS + 8 * u), 8), :] = (e >> 16) | (o & jnp.uint32(0xFFFF0000))
                return c2
            lax.fori_loop(0, ng // ux, inner, 0)
            return carry
        lax.fori_loop(0, 4, body, 0)

    def phase_fv(q):
        b = q >> 1

        def body(it, carry):
            dmat = _as_bf16(d_ref[...])
            zero = ZV[...]
            jp0 = it * UF
            xsb = b * XS_ROWS + 64 * jp0
            xhb = b * 32 + jp0
            npos = 4
            pos0 = 8 * b + it * npos
            em = _Emitter(_v_units(wview(1, pos0 * 8, npos * 8), SC, WH0, pos0 * (192 * 8), 0, npos, do2=False))
            nd, di = UF * 8, 0
            for u in range(UF):
                for p in range(2):
                    for ct in range(4):
                        off = (p * 8 + ct * 2) * XS_ROWS + 64 * u
                        t0 = _pad64(XS[pl.ds(xsb + off, 48), :])
                        t1 = _pad64(XS[pl.ds(xsb + off + 32, 48), :])
                        r0 = jnp.dot(dmat, _as_bf16(t0), preferred_element_type=F32)
                        r1 = jnp.dot(dmat, _as_bf16(t1), preferred_element_type=F32)
                        for fg in range(6):
                            xr0, xi0 = r0[16 * fg:16 * fg + 8], r0[16 * fg + 8:16 * fg + 16]
                            xr1, xi1 = r1[16 * fg:16 * fg + 8], r1[16 * fg + 8:16 * fg + 16]
                            for op, val in ((0, _pack(xr0, xr1)), (1, _pack(xr0 + xi0, xr1 + xi1)),
                                            (2, _pack(xi0 - xr0, xi1 - xr1))):
                                a = ((op * 4 + ct) * F + 8 * fg) * PX + p * 16 + u
                                XH[pl.ds(xhb + a, 8, stride=PX), :] = val
                        di += 1
                        _Dep.v = lax.bitcast_convert_type(r0[0:8], U32) & zero
                        em.upto(di / nd)
            em.upto(2.0)
            _Dep.v = None
            return carry
        lax.fori_loop(q & 1, (q & 1) + 1, body, 0)

    def dma_half(s, half):
        if half == 0:
            @pl.when(s + 1 <= 7)
            def _():
                wh_copy(s + 1, 1, _mod3(s + 1)).wait()

            @pl.when(s + 3 <= 7)
            def _():
                wh_copy(s + 3, 0, _mod3(s)).start()
                wh_copy(s + 3, 1, _mod3(s)).start()
        else:
            @pl.when(s + 2 <= 7)
            def _():
                wh_copy(s + 2, 0, _mod3(s + 2)).wait()

    def phase_pv(s, WHr, WHw, ybase):
        slot1 = _mod3(s + 1)
        slot2 = _mod3(s + 2)

        def body(it, c):
            f0 = it * UP
            xb, wb, yb = f0 * PX, f0 * PW, ybase + f0
            last = it == NIT - 1
            g1 = jnp.where(last, 0, it + 1)
            cpg = it * (NP * 8)
            whb = (cpg >> 6) * (F * PW) + (cpg & 63)
            em = _Emitter(_v_units(wview(jnp.where(last, slot2, slot1), g1 * (NP * 8), NP * 8),
                                   SC, WHw, 0, whb, NP), VLEAD)
            nd = UP * 12 * MH
            di = 0
            MR = 64 // MH
            for u in range(UP):
                for hh in range(MH):
                    ks = {}
                    for op in (1, 2, 0):
                        ds = []
                        for kt in (0, 2, 1, 3):
                            xa = ((op * 4 + kt) * F + u) * PX + hh * MR
                            wa = ((op * 4 + kt) * F + u) * PW
                            ds.append(jnp.dot(_as_bf16(XH[pl.ds(xb + xa, MR), :]),
                                              _as_bf16(WHr[pl.ds(wb + wa, 64), :]), preferred_element_type=F32))
                            di += 1
                            em.upto(di / nd)
                        ks[op] = (ds[0] + ds[1]) + (ds[2] + ds[3])
                    y = _pack(ks[0] - ks[1], ks[0] + ks[2])
                    for i in range(16 // MH):
                        YH[pl.ds(yb + ((8 * i + hh * 2 * MR) * PY + u), 8, stride=PY), :] = y[8 * i:8 * i + 8]
            em.upto(2.0)
            return c

        def half_step(hs, c):
            @pl.when(hs == 0)
            def _():
                dma_half(s, 0)

            @pl.when(hs == 1)
            def _():
                dma_half(s, 1)
            lax.fori_loop(hs, hs + 1, body, 0)
            return c
        lax.fori_loop(0, NIT, half_step, 0)

    def phase_i(ct):
        cmat = _as_bf16(c_ref[...])
        for u in range(64):
            hs = {}
            b, j = u >> 5, u & 31
            for p in range(2):
                for tl in range(2):
                    yb = (b * 64 + j) * PY
                    rhs = _as_bf16(_pad64(YH[pl.ds(yb + (tl * YH_ROWS + p * 32 * PY), 48), :]))
                    hs[p, tl] = jnp.dot(cmat, rhs, preferred_element_type=F32)
            zs = [jnp.tanh(hs[p, 0]) * (0.5 * jnp.tanh(0.5 * hs[p, 1]) + 0.5) for p in range(2)]
            ZB[pl.ds(ct * 4096 + b * 2048 + 64 * j, 64), :] = _pack(zs[0], zs[1])

    def p1_loop(u0, u1):
        def body(u, carry):
            for g in _v_units(wview(0, u * 8, 8), SC, WH0, u * (192 * 8), 0, 1, do2=False):
                next(g)
            return carry
        lax.fori_loop(u0, u1, body, 0)

    w0_copy(0, 32, 6).wait()
    p1_loop(0, 2)
    w0_copy(32, 96, 14).wait()
    p1_loop(2, 8)
    xq_start(1)

    def vonly(g, carry):
        _Emitter(_v_units(wview(0, (g + 1) * 64, 64), SC, WH0, 0, g * (F * PW), 8)).upto(2.0)
        return carry

    def vstep(g, carry):
        w0_copy((g + 1) * 128, 128, 7 + g).wait()
        lax.fori_loop(g, g + 1, vonly, 0)

        @pl.when(g == 0)
        def _():
            xq_start(2)

        @pl.when(g == 1)
        def _():
            xq_start(3)
            wh_copy(1, 1, 1).start()
        return carry
    lax.fori_loop(0, 3, vstep, 0)
    _Emitter(_v_units(None, SC, WH0, 0, 3 * (F * PW), 8, do1=False)).upto(2.0)

    def qstep(q, carry):
        b = q >> 1
        for h in range(2):
            @pl.when((q & 1) == h)
            def _():
                for ct in range(4):
                    x_copy(ct, b, h).wait()
                phase_xs(b, h)
        w1_copy(q).wait()

        @pl.when(q == 1)
        def _():
            wh_copy(2, 0, 2).start()
            wh_copy(2, 1, 2).start()
        phase_fv(q)
        return carry
    lax.fori_loop(0, 4, qstep, 0)
    for nt in range(4):
        wo_copy(nt).start()

    def step2(c, carry):
        s = 2 * c
        phase_pv(s, WH0, WH1, 0)
        phase_pv(s + 1, WH1, WH0, YH_ROWS)
        phase_i(c)
        return carry
    lax.fori_loop(0, 4, step2, 0)

    for nt in range(4):
        wo_copy(nt).wait()
    nblk = T // OB_ROWS

    def wait_out(par):
        for u in range(UO - 1):
            o_copy(par * UO + u, 0, 0, par).wait()
        for nt in range(4):
            o_copy(par * UO + UO - 1, 0, 0, par, nt).wait()

    def obody(it, carry):
        par = it & 1

        @pl.when(it >= 2)
        def _():
            wait_out(par)
        for u in range(UO):
            idx = it * UO + u
            b = (idx >= nblk).astype(jnp.int32)
            blk = idx - b * nblk
            slot = par * UO + u
            zb = b * 2048 + blk * (OB_ROWS // 2)
            lhs = [_as_bf16(ZB[pl.ds(zb + ct * 4096, OB_ROWS // 2), :]) for ct in range(4)]
            for nt in range(4):
                acc = None
                for kt in range(4):
                    d = jnp.dot(lhs[kt], _as_bf16(WO[pl.ds(nt * 256 + kt * 64, 64), :]),
                                preferred_element_type=F32)
                    acc = d if acc is None else acc + d
                OB[slot, :, pl.ds(nt * 128, 128)] = acc.astype(BF)
                if u == UO - 1:
                    o_copy(slot, b, blk, par, nt).start()
            if u < UO - 1:
                o_copy(slot, b, blk, par).start()
        return carry
    lax.fori_loop(0, B * nblk // UO, obody, 0)
    for par in range(2):
        wait_out(par)


def make_fft(name="wavenet_fft_conv"):
    def fn(x, w, w_o):
        scratch = [
            pltpu.VMEM((8 * XW_ROWS, 128), U32),
            pltpu.VMEM((16 * XS_ROWS, 128), U32),
            pltpu.VMEM((12 * F * PX + 64, 128), U32),
            pltpu.VMEM((3 * K, D, 128), BF),
            pltpu.VMEM((12 * F * PW, 128), U32),
            pltpu.VMEM((12 * F * PW, 128), U32),
            pltpu.VMEM((16 * 192 * 8, 128), F32),
            pltpu.VMEM((2 * YH_ROWS + 64, 128), U32),
            pltpu.VMEM((8 * 2048, 128), U32),
            pltpu.VMEM((4 * 256, 128), U32),
            pltpu.VMEM((2 * UO, OB_ROWS, D), BF),
            pltpu.VMEM((8, 128), U32),
            pltpu.SemaphoreType.DMA((4,)), pltpu.SemaphoreType.DMA((15,)), pltpu.SemaphoreType.DMA,
            pltpu.SemaphoreType.DMA((2,)),
        ]
        return pl.pallas_call(
            _kernel,
            out_shape=jax.ShapeDtypeStruct((B, T, D), BF),
            in_specs=[pl.BlockSpec(memory_space=pltpu.VMEM)] * 2 + [pl.BlockSpec(memory_space=pl.ANY)] * 3,
            out_specs=pl.BlockSpec(memory_space=pl.ANY),
            scratch_shapes=scratch,
            compiler_params=pltpu.CompilerParams(vmem_limit_bytes=126 * 1024 * 1024),
            name=name,
        )(jnp.asarray(_DMAT), jnp.asarray(_CMAT), x, w, w_o)
    fn.__name__ = name
    return fn


@jax.jit
def pallas_standalone__autoregressive_conv_wavenet__speech_kernel(
    x: jax.Array,
    w: jax.Array,
    w_o: jax.Array,
):
    assert x.shape == (B, T, D) and w.shape == (K, D, 2 * D) and w_o.shape == (D, D)
    return make_fft()(x, w, w_o)
```
